```python
import jax
import jax.numpy as jnp

def _softmax(x, axis=-1):
    return jax.nn.softmax(x, axis=axis)
def _gelu(x):
    return jax.nn.gelu(x, approximate=True)
def _silu(x):
    return jax.nn.silu(x)
def _sigmoid(x):
    return jax.nn.sigmoid(x)
def _layernorm(x, axis=-1, eps=1e-5):
    m = jnp.mean(x, axis=axis, keepdims=True)
    v = jnp.var(x, axis=axis, keepdims=True)
    return (x - m) / jnp.sqrt(v + eps)
def _scatter_add(tgt, idx, src, axis=0):
    return tgt.at[idx].add(src)
def _segment_sum(src, seg, n):
    return jax.ops.segment_sum(src, seg, n)
class _Rng:
    def __init__(self, key):
        self._k = key
    def _next(self):
        self._k, sub = jax.random.split(self._k)
        return sub
    def normal(self, shape):
        return jax.random.normal(self._next(), shape, dtype=jnp.bfloat16)
    def randint(self, lo, hi, shape):
        return jax.random.randint(self._next(), shape, lo, hi, dtype=jnp.int32)
    def uniform(self, shape, lo=0.0, hi=1.0):
        return jax.random.uniform(self._next(), shape, jnp.bfloat16, lo, hi)
    def permutation(self, n):
        return jax.random.permutation(self._next(), n)


kernel_name = 'recurrent_scan__compressed_kv_cla__dense_activation_silu__decode'

def setup_inputs():
    _rng = _Rng(jax.random.key(int.from_bytes(__import__("os").urandom(4), "little")))
    _w = (lambda a: (lambda t: t.astype(jnp.bfloat16) if jnp.issubdtype(t.dtype, jnp.floating) else t)(jnp.asarray(a)))
    def _A_setup():
        B, H, Sq, Sk, D, M = 1, 32, 1, 32768, 128, 512
        Dc = 4 * D
        return {
            "x": _w((lambda *s: _rng.normal(s) * 0.05)(B, Sq, M)),
            "c_kv": _w((lambda *s: _rng.normal(s) * 0.05)(B, Sk, Dc)),
            "w_q": _w((lambda *s: _rng.normal(s) * 0.05)(M, H, D) * (M ** -0.5)),
            "w_uk": _w((lambda *s: _rng.normal(s) * 0.05)(Dc, H, D) * (Dc ** -0.5)),
            "w_uv": _w((lambda *s: _rng.normal(s) * 0.05)(Dc, H, D) * (Dc ** -0.5)),
            "w_o": _w((lambda *s: _rng.normal(s) * 0.05)(H, D, M) * ((H * D) ** -0.5)),
        }
    _A_in = _A_setup()

    def _B_setup():
        B, S, D, F = 1, 1, 512, 1376
        return {
            "x": _w((lambda *s: _rng.normal(s) * 0.05)(B, S, D)),
            "w1": _w((lambda *s: _rng.normal(s) * 0.05)(D, F) * (D ** -0.5)),
            "w2": _w((lambda *s: _rng.normal(s) * 0.05)(F, D) * (F ** -0.5)),
        }
    _B_in = _B_setup()

    return {
        "A_x": _A_in["x"],
        "A_c_kv": _A_in["c_kv"],
        "A_w_q": _A_in["w_q"],
        "A_w_uk": _A_in["w_uk"],
        "A_w_uv": _A_in["w_uv"],
        "A_w_o": _A_in["w_o"],
        "B_x": _B_in["x"],
        "B_w1": _B_in["w1"],
        "B_w2": _B_in["w2"],
    }

def reference(A_x, A_c_kv, A_w_q, A_w_uk, A_w_uv, A_w_o, B_x, B_w1, B_w2):
    def _A_ref(x, c_kv, w_q, w_uk, w_uv, w_o):
        B, Sq, M = x.shape[0], x.shape[1], x.shape[2]
        Sk = c_kv.shape[1]
        H, D = w_q.shape[1], w_q.shape[2]
        q = jnp.einsum("bqm,mhd->bhqd", x, w_q)
        k = jnp.einsum("bkc,chd->bhkd", c_kv, w_uk)
        v = jnp.einsum("bkc,chd->bhkd", c_kv, w_uv)
        scores = jnp.einsum("bhqd,bhkd->bhqk", q, k) * (D ** -0.5)
        off = Sk - Sq
        qi = jnp.arange(Sq)[:, None]
        kj = jnp.arange(Sk)[None, :]
        cmask = kj <= (qi + off)
        scores = jnp.where(cmask[None, None], scores, -1e9)
        p = _softmax(scores, axis=-1)
        ctx = jnp.einsum("bhqk,bhkd->bhqd", p, v)
        return jnp.einsum("bhqd,hdm->bqm", ctx, w_o)

    def _B_ref(x, w1, w2):
        h = jnp.einsum("bsd,df->bsf", x, w1)
        h = _silu(h)
        out = jnp.einsum("bsf,fd->bsd", h, w2)
        return out

    x = A_x
    xn = _layernorm(x, axis=-1)
    s = _A_ref(xn, A_c_kv, A_w_q, A_w_uk, A_w_uv, A_w_o)
    g = _silu(_B_ref(xn, B_w1, B_w2))
    return x + s * g
```

```python
import jax
import jax.numpy as jnp
from jax import lax
import jax.experimental.pallas as pl
import jax.experimental.pallas.tpu as pltpu

M = 512
H = 32
D = 128
C = 512
SK = 32768
F = 1376

T = 2048
NDMA = 4
G = 8
WO_CHUNKS = (24, 5, 2, 1)

F32 = jnp.float32
BF16 = jnp.bfloat16
LOG2E = 1.4426950408889634


def _kernel(x_hbm, ckv_hbm, wq_hbm, wuk_hbm, wuv_hbm, wo_hbm, w1_hbm, w2_hbm, o_ref,
            x_s, ckv_s, wq_s, wuk_s, wuv_s, wo_s, w1_s, w2_s, v_s, qa_s, sems):
    NKV = SK // T
    SUB = NKV // NDMA
    TD = SK // NDMA

    cp_x = pltpu.make_async_copy(x_hbm, x_s, sems.at[0])
    cp_q = pltpu.make_async_copy(wq_hbm, wq_s, sems.at[1])
    cp_uk = pltpu.make_async_copy(wuk_hbm, wuk_s, sems.at[2])
    cp_w1 = pltpu.make_async_copy(w1_hbm, w1_s, sems.at[3])
    cp_w2 = pltpu.make_async_copy(w2_hbm, w2_s, sems.at[4])
    cp_uv = pltpu.make_async_copy(wuv_hbm, wuv_s, sems.at[5])

    def cp_kv(i):
        return pltpu.make_async_copy(ckv_hbm.at[pl.ds(i * TD, TD)], ckv_s.at[pl.ds(i * TD, TD)], sems.at[6 + i])

    wo_offs = []
    off = 0
    for n in WO_CHUNKS:
        wo_offs.append((off, n))
        off += n

    def cp_wo(k):
        o, n = wo_offs[k]
        return pltpu.make_async_copy(wo_hbm.at[pl.ds(o, n)], wo_s.at[pl.ds(o, n)], sems.at[6 + NDMA + k])

    cp_x.start(); cp_q.start(); cp_uk.start(); cp_w1.start(); cp_w2.start()
    for i in range(NDMA):
        cp_kv(i).start()
    cp_uv.start()
    for k in range(len(WO_CHUNKS)):
        cp_wo(k).start()

    cp_x.wait()
    x = x_s[...].astype(F32)
    mu = jnp.mean(x, axis=-1, keepdims=True)
    xc = x - mu
    var = jnp.mean(xc * xc, axis=-1, keepdims=True)
    xn = (xc / jnp.sqrt(var + 1e-5)).astype(BF16)
    xn32 = xn.astype(F32)

    lane_h = lax.broadcasted_iota(jnp.int32, (H, 128), 1) % H
    row_h = lax.broadcasted_iota(jnp.int32, (H, 128), 0)
    dmask = lane_h == row_h
    xrt = jnp.concatenate([jnp.broadcast_to(xn32[:, 128 * i:128 * (i + 1)], (H, 128)) for i in range(4)], axis=0)
    v_s[...] = xrt.T

    def w_tile(w_ref, j):
        return w_ref[:, pl.ds(j, 1)].reshape(4 * H, D)

    def contract_rows(w_ref):
        def body(g, acc):
            j0 = pl.multiple_of(g * G, G)
            vg = v_s[pl.ds(j0, G), :]
            for s in range(G):
                xj = jnp.where(dmask, jnp.broadcast_to(vg[s:s + 1, :], (H, 128)), 0.0).astype(BF16)
                acc = acc + jnp.dot(xj, w_tile(w_ref, j0 + s), preferred_element_type=F32)
            return acc
        return lax.fori_loop(0, 128 // G, body, jnp.zeros((H, D), F32))

    cp_q.wait()
    q = contract_rows(wq_s).astype(BF16)

    cp_uk.wait()

    def qa_body(g, carry):
        j0 = pl.multiple_of(g * G, G)
        rows = []
        for s in range(G):
            o = lax.dot_general(q, w_tile(wuk_s, j0 + s), (((1,), (1,)), ((), ())), preferred_element_type=F32)
            rows.append(jnp.sum(jnp.where(dmask, o, 0.0), axis=0, keepdims=True))
        v_s[pl.ds(j0, G), :] = jnp.concatenate(rows, axis=0)
        return carry
    lax.fori_loop(0, 128 // G, qa_body, 0)
    vt = v_s[...].T
    for i in range(4):
        qa_s[:, 128 * i:128 * (i + 1)] = vt[H * i:H * (i + 1), :].astype(BF16)

    cp_w1.wait()
    h1 = lax.dot_general(xn, w1_s[...], (((1,), (1,)), ((), ())), preferred_element_type=F32)
    h1 = h1.astype(BF16).astype(F32)
    a1 = (h1 * jax.nn.sigmoid(h1)).astype(BF16)
    cp_w2.wait()
    f2 = jnp.dot(a1, w2_s[...], preferred_element_type=F32)
    f2 = f2.astype(BF16).astype(F32)
    gate = f2 * jax.nn.sigmoid(f2)

    sc = (D ** -0.5) * LOG2E

    def att_body(i, carry):
        m, l, acc = carry

        @pl.when(i % SUB == 0)
        def _():
            cp_kv(i // SUB).wait()

        blk = ckv_s[pl.ds(pl.multiple_of(i * T, T), T), :]
        s = lax.dot_general(qa_s[...], blk, (((1,), (1,)), ((), ())), preferred_element_type=F32) * sc
        m_new = jnp.maximum(m, jnp.max(s, axis=1, keepdims=True))
        p = jnp.exp2(s - m_new)
        alpha = jnp.exp2(m - m_new)
        l = alpha * l + jnp.sum(p, axis=1, keepdims=True)
        acc = alpha * acc + jnp.dot(p.astype(BF16), blk, preferred_element_type=F32)
        return m_new, l, acc

    m, l, acc = lax.fori_loop(0, NKV, att_body,
                              (jnp.full((H, 1), -1e30, F32), jnp.zeros((H, 1), F32), jnp.zeros((H, C), F32)))
    olat = acc / l
    vt = jnp.concatenate([olat[:, 128 * i:128 * (i + 1)] for i in range(4)], axis=0)
    v_s[...] = vt.T

    cp_uv.wait()
    ctx = contract_rows(wuv_s).astype(BF16)

    s_acc = jnp.zeros((1, M), F32)
    for k, (o, n) in enumerate(wo_offs):
        cp_wo(k).wait()
        for h in range(o, o + n):
            s_acc = s_acc + jnp.dot(ctx[h:h + 1, :], wo_s[h], preferred_element_type=F32)
    o_ref[...] = (x + s_acc * gate).astype(o_ref.dtype)


@jax.jit
def pallas_recurrent_scan__compressed_kv_cla__dense_activation_silu__decode_kernel(
    A_x: jax.Array,
    A_c_kv: jax.Array,
    A_w_q: jax.Array,
    A_w_uk: jax.Array,
    A_w_uv: jax.Array,
    A_w_o: jax.Array,
    B_x: jax.Array,
    B_w1: jax.Array,
    B_w2: jax.Array,
):
    del B_x
    any_spec = pl.BlockSpec(memory_space=pl.ANY)
    out = pl.pallas_call(
        _kernel,
        in_specs=[any_spec] * 8,
        out_specs=pl.BlockSpec(memory_space=pltpu.VMEM),
        out_shape=jax.ShapeDtypeStruct((1, M), BF16),
        scratch_shapes=[
            pltpu.VMEM((1, M), BF16),
            pltpu.VMEM((SK, C), BF16),
            pltpu.VMEM((4, 128, H, D), BF16),
            pltpu.VMEM((4, 128, H, D), BF16),
            pltpu.VMEM((4, 128, H, D), BF16),
            pltpu.VMEM((H, D, M), BF16),
            pltpu.VMEM((F, M), BF16),
            pltpu.VMEM((F, M), BF16),
            pltpu.VMEM((128, 128), F32),
            pltpu.VMEM((H, C), BF16),
            pltpu.SemaphoreType.DMA((6 + NDMA + len(WO_CHUNKS),)),
        ],
        compiler_params=pltpu.CompilerParams(vmem_limit_bytes=100 * 1024 * 1024),
    )(A_x.reshape(1, M), A_c_kv.reshape(SK, C), A_w_q.reshape(4, 128, H, D), A_w_uk.reshape(4, 128, H, D),
      A_w_uv.reshape(4, 128, H, D), A_w_o, B_w1.T, B_w2)
    return out.reshape(1, 1, M)
```

```python
import jax
import jax.numpy as jnp
from jax import lax
import jax.experimental.pallas as pl
import jax.experimental.pallas.tpu as pltpu

M = 512
H = 32
D = 128
C = 512
SK = 32768
F = 1376

T = 2048
NDMA = 4
G = 8
WO_MXU = (24, 5, 2)

F32 = jnp.float32
BF16 = jnp.bfloat16
LOG2E = 1.4426950408889634
NSEM = 6 + NDMA + len(WO_MXU) + 1


def _silu(v):
    return v * jax.nn.sigmoid(v)


def _kernel(x_hbm, ckv_hbm, wq_hbm, wuk_hbm, wuv_hbm, wo_hbm, w1t_hbm, w2_hbm, o_ref,
            x_s, ckv_s, wq_s, wuk_s, wuv_s, wo_s, w1t_s, w2_s, v_s, qa_s, sems):
    steps_per_dma = SK // T // NDMA
    rows_per_dma = SK // NDMA

    cp_q = pltpu.make_async_copy(wq_hbm, wq_s, sems.at[0])
    cp_x = pltpu.make_async_copy(x_hbm, x_s, sems.at[1])
    cp_uk = pltpu.make_async_copy(wuk_hbm, wuk_s, sems.at[2])
    cp_w1 = pltpu.make_async_copy(w1t_hbm, w1t_s, sems.at[3])
    cp_w2 = pltpu.make_async_copy(w2_hbm, w2_s, sems.at[4])
    cp_uv = pltpu.make_async_copy(wuv_hbm, wuv_s, sems.at[5])

    def cp_kv(i):
        rows = pl.ds(i * rows_per_dma, rows_per_dma)
        return pltpu.make_async_copy(ckv_hbm.at[rows], ckv_s.at[rows], sems.at[6 + i])

    wo_heads = []
    h0 = 0
    for n in WO_MXU + (1,):
        wo_heads.append((h0, n))
        h0 += n
    assert h0 == H

    def cp_wo(k):
        h, n = wo_heads[k]
        rows = pl.ds(h * D, n * D)
        return pltpu.make_async_copy(wo_hbm.at[rows], wo_s.at[rows], sems.at[6 + NDMA + k])

    cp_q.start()
    cp_x.start()
    cp_uk.start()
    cp_w1.start()
    cp_w2.start()
    for i in range(NDMA):
        cp_kv(i).start()
    cp_uv.start()
    for k in range(len(wo_heads)):
        cp_wo(k).start()

    cp_x.wait()
    x = x_s[...].astype(F32)
    mu = jnp.mean(x, axis=-1, keepdims=True)
    xc = x - mu
    var = jnp.mean(xc * xc, axis=-1, keepdims=True)
    xn = (xc / jnp.sqrt(var + 1e-5)).astype(BF16)

    lane_head = lax.broadcasted_iota(jnp.int32, (H, 128), 1) % H
    row_head = lax.broadcasted_iota(jnp.int32, (H, 128), 0)
    head_mask = lane_head == row_head

    def w_tile(w_ref, j):
        return w_ref[:, pl.ds(j, 1)].reshape(4 * H, D)

    def contract_c(w_ref):
        def body(g, acc):
            j0 = pl.multiple_of(g * G, G)
            vg = v_s[pl.ds(j0, G), :]
            for s in range(G):
                lhs = jnp.where(head_mask, jnp.broadcast_to(vg[s:s + 1, :], (H, 128)), 0.0).astype(BF16)
                acc = acc + jnp.dot(lhs, w_tile(w_ref, j0 + s), preferred_element_type=F32)
            return acc
        return lax.fori_loop(0, 128 // G, body, jnp.zeros((H, D), F32))

    xn32 = xn.astype(F32)
    vt = jnp.concatenate(
        [jnp.broadcast_to(xn32[:, 128 * i:128 * (i + 1)], (H, 128)) for i in range(4)], axis=0)
    v_s[...] = vt.T
    cp_q.wait()
    q = contract_c(wq_s).astype(BF16)

    cp_uk.wait()

    def absorb_body(g, carry):
        j0 = pl.multiple_of(g * G, G)
        rows = []
        for s in range(G):
            full = lax.dot_general(q, w_tile(wuk_s, j0 + s), (((1,), (1,)), ((), ())),
                                   preferred_element_type=F32)
            rows.append(jnp.sum(jnp.where(head_mask, full, 0.0), axis=0, keepdims=True))
        v_s[pl.ds(j0, G), :] = jnp.concatenate(rows, axis=0)
        return carry

    lax.fori_loop(0, 128 // G, absorb_body, 0)
    vt = v_s[...].T
    for i in range(4):
        qa_s[:, 128 * i:128 * (i + 1)] = vt[H * i:H * (i + 1), :].astype(BF16)

    cp_w1.wait()
    h1 = lax.dot_general(xn, w1t_s[...], (((1,), (1,)), ((), ())), preferred_element_type=F32)
    a1 = _silu(h1.astype(BF16).astype(F32)).astype(BF16)
    cp_w2.wait()
    f2 = jnp.dot(a1, w2_s[...], preferred_element_type=F32)
    gate = _silu(f2.astype(BF16).astype(F32))

    scale = (D ** -0.5) * LOG2E

    def att_body(i, carry):
        m, l, acc = carry

        @pl.when(i % steps_per_dma == 0)
        def _():
            cp_kv(i // steps_per_dma).wait()

        blk = ckv_s[pl.ds(pl.multiple_of(i * T, T), T), :]
        s = lax.dot_general(qa_s[...], blk, (((1,), (1,)), ((), ())),
                            preferred_element_type=F32) * scale
        m_new = jnp.maximum(m, jnp.max(s, axis=1, keepdims=True))
        p = jnp.exp2(s - m_new)
        alpha = jnp.exp2(m - m_new)
        l = alpha * l + jnp.sum(p, axis=1, keepdims=True)
        acc = alpha * acc + jnp.dot(p.astype(BF16), blk, preferred_element_type=F32)
        return m_new, l, acc

    _, l, acc = lax.fori_loop(
        0, SK // T, att_body,
        (jnp.full((H, 1), -jnp.inf, F32), jnp.zeros((H, 1), F32), jnp.zeros((H, C), F32)))
    o_lat = acc / l
    vt = jnp.concatenate([o_lat[:, 128 * i:128 * (i + 1)] for i in range(4)], axis=0)
    v_s[...] = vt.T

    cp_uv.wait()
    ctx = contract_c(wuv_s).astype(BF16)
    ctx_t = jnp.concatenate([ctx.astype(F32)] * 4, axis=0).T
    ctx_last = jnp.broadcast_to(ctx_t[:, H - 1:H], (D, 128))

    s_acc = jnp.zeros((1, M), F32)
    for k in range(len(WO_MXU)):
        h0, n = wo_heads[k]
        cp_wo(k).wait()
        for h in range(h0, h0 + n):
            s_acc = s_acc + jnp.dot(ctx[h:h + 1, :], wo_s[h * D:(h + 1) * D, :],
                                    preferred_element_type=F32)
    base = x + s_acc * gate
    cp_wo(len(WO_MXU)).wait()
    blk = wo_s[(H - 1) * D:H * D, :].astype(F32)
    s_last = jnp.concatenate(
        [jnp.sum(blk[:, 128 * j:128 * (j + 1)] * ctx_last, axis=0, keepdims=True) for j in range(4)],
        axis=1)
    o_ref[...] = (base + s_last * gate).astype(o_ref.dtype)


@jax.jit
def pallas_recurrent_scan__compressed_kv_cla__dense_activation_silu__decode_kernel(
    A_x: jax.Array,
    A_c_kv: jax.Array,
    A_w_q: jax.Array,
    A_w_uk: jax.Array,
    A_w_uv: jax.Array,
    A_w_o: jax.Array,
    B_x: jax.Array,
    B_w1: jax.Array,
    B_w2: jax.Array,
):
    del B_x
    any_spec = pl.BlockSpec(memory_space=pl.ANY)
    w_shape = (4, 128, H, D)
    out = pl.pallas_call(
        _kernel,
        in_specs=[any_spec] * 8,
        out_specs=pl.BlockSpec(memory_space=pltpu.VMEM),
        out_shape=jax.ShapeDtypeStruct((1, M), BF16),
        scratch_shapes=[
            pltpu.VMEM((1, M), BF16),
            pltpu.VMEM((SK, C), BF16),
            pltpu.VMEM(w_shape, BF16),
            pltpu.VMEM(w_shape, BF16),
            pltpu.VMEM(w_shape, BF16),
            pltpu.VMEM((H * D, M), BF16),
            pltpu.VMEM((F, M), BF16),
            pltpu.VMEM((F, M), BF16),
            pltpu.VMEM((128, 128), F32),
            pltpu.VMEM((H, C), BF16),
            pltpu.SemaphoreType.DMA((NSEM,)),
        ],
        compiler_params=pltpu.CompilerParams(
            vmem_limit_bytes=80 * 1024 * 1024,
            disable_bounds_checks=True,
            disable_semaphore_checks=True,
        ),
    )(
        A_x.reshape(1, M),
        A_c_kv.reshape(SK, C),
        A_w_q.reshape(w_shape),
        A_w_uk.reshape(w_shape),
        A_w_uv.reshape(w_shape),
        A_w_o.reshape(H * D, M),
        B_w1.T,
        B_w2,
    )
    return out.reshape(1, 1, M)
```

```python
import jax
import jax.numpy as jnp
from jax import lax
import jax.experimental.pallas as pl
import jax.experimental.pallas.tpu as pltpu

M = 512
H = 32
D = 128
C = 512
SK = 32768
F = 1376

T = 2048
NDMA = 4
G = 8
WO_MXU = (24, 5, 2)
WO_VPU = (96, 32)

F32 = jnp.float32
BF16 = jnp.bfloat16
LOG2E = 1.4426950408889634
NSEM = 6 + NDMA + len(WO_MXU) + len(WO_VPU)


def _silu(v):
    return v * jax.nn.sigmoid(v)


def _kernel(x_hbm, ckv_hbm, wq_hbm, wuk_hbm, wuv_hbm, wo_hbm, w1t_hbm, w2_hbm, o_ref,
            x_s, ckv_s, wq_s, wuk_s, wuv_s, wo_s, w1t_s, w2_s, v_s, qa_s, sems):
    steps_per_dma = SK // T // NDMA
    rows_per_dma = SK // NDMA

    cp_q = pltpu.make_async_copy(wq_hbm, wq_s, sems.at[0])
    cp_x = pltpu.make_async_copy(x_hbm, x_s, sems.at[1])
    cp_uk = pltpu.make_async_copy(wuk_hbm, wuk_s, sems.at[2])
    cp_w1 = pltpu.make_async_copy(w1t_hbm, w1t_s, sems.at[3])
    cp_w2 = pltpu.make_async_copy(w2_hbm, w2_s, sems.at[4])
    cp_uv = pltpu.make_async_copy(wuv_hbm, wuv_s, sems.at[5])

    def cp_kv(i):
        rows = pl.ds(i * rows_per_dma, rows_per_dma)
        return pltpu.make_async_copy(ckv_hbm.at[rows], ckv_s.at[rows], sems.at[6 + i])

    wo_rows = []
    r0 = 0
    for n in tuple(h * D for h in WO_MXU) + WO_VPU:
        wo_rows.append((r0, n))
        r0 += n
    assert r0 == H * D and sum(WO_VPU) == D

    def cp_wo(k):
        rows = pl.ds(*wo_rows[k])
        return pltpu.make_async_copy(wo_hbm.at[rows], wo_s.at[rows], sems.at[6 + NDMA + k])

    cp_q.start()
    cp_x.start()
    cp_uk.start()
    cp_w1.start()
    cp_w2.start()
    for i in range(NDMA):
        cp_kv(i).start()
    cp_uv.start()
    for k in range(len(wo_rows)):
        cp_wo(k).start()

    cp_x.wait()
    x = x_s[...].astype(F32)
    mu = jnp.mean(x, axis=-1, keepdims=True)
    xc = x - mu
    var = jnp.mean(xc * xc, axis=-1, keepdims=True)
    xn = (xc / jnp.sqrt(var + 1e-5)).astype(BF16)

    lane_head = lax.broadcasted_iota(jnp.int32, (H, 128), 1) % H
    row_head = lax.broadcasted_iota(jnp.int32, (H, 128), 0)
    head_mask = lane_head == row_head

    def w_tile(w_ref, j):
        return w_ref[:, pl.ds(j, 1)].reshape(4 * H, D)

    def contract_c(w_ref):
        def body(g, acc):
            j0 = pl.multiple_of(g * G, G)
            vg = v_s[pl.ds(j0, G), :]
            for s in range(G):
                lhs = jnp.where(head_mask, jnp.broadcast_to(vg[s:s + 1, :], (H, 128)), 0.0).astype(BF16)
                acc = acc + jnp.dot(lhs, w_tile(w_ref, j0 + s), preferred_element_type=F32)
            return acc
        return lax.fori_loop(0, 128 // G, body, jnp.zeros((H, D), F32))

    xn32 = xn.astype(F32)
    vt = jnp.concatenate(
        [jnp.broadcast_to(xn32[:, 128 * i:128 * (i + 1)], (H, 128)) for i in range(4)], axis=0)
    v_s[...] = vt.T
    cp_q.wait()
    q = contract_c(wq_s).astype(BF16)

    cp_uk.wait()

    def absorb_body(g, carry):
        j0 = pl.multiple_of(g * G, G)
        rows = []
        for s in range(G):
            full = lax.dot_general(q, w_tile(wuk_s, j0 + s), (((1,), (1,)), ((), ())),
                                   preferred_element_type=F32)
            rows.append(jnp.sum(jnp.where(head_mask, full, 0.0), axis=0, keepdims=True))
        v_s[pl.ds(j0, G), :] = jnp.concatenate(rows, axis=0)
        return carry

    lax.fori_loop(0, 128 // G, absorb_body, 0)
    vt = v_s[...].T
    for i in range(4):
        qa_s[:, 128 * i:128 * (i + 1)] = vt[H * i:H * (i + 1), :].astype(BF16)

    cp_w1.wait()
    h1 = lax.dot_general(xn, w1t_s[...], (((1,), (1,)), ((), ())), preferred_element_type=F32)
    a1 = _silu(h1.astype(BF16).astype(F32)).astype(BF16)
    cp_w2.wait()
    f2 = jnp.dot(a1, w2_s[...], preferred_element_type=F32)
    gate = _silu(f2.astype(BF16).astype(F32))

    scale = (D ** -0.5) * LOG2E

    def att_body(i, carry):
        m, l, acc = carry

        @pl.when(i % steps_per_dma == 0)
        def _():
            cp_kv(i // steps_per_dma).wait()

        blk = ckv_s[pl.ds(pl.multiple_of(i * T, T), T), :]
        s = lax.dot_general(qa_s[...], blk, (((1,), (1,)), ((), ())),
                            preferred_element_type=F32) * scale
        m_new = jnp.maximum(m, jnp.max(s, axis=1, keepdims=True))
        p = jnp.exp2(s - m_new)
        alpha = jnp.exp2(m - m_new)
        l = alpha * l + jnp.sum(p, axis=1, keepdims=True)
        acc = alpha * acc + jnp.dot(p.astype(BF16), blk, preferred_element_type=F32)
        return m_new, l, acc

    _, l, acc = lax.fori_loop(
        0, SK // T, att_body,
        (jnp.full((H, 1), -jnp.inf, F32), jnp.zeros((H, 1), F32), jnp.zeros((H, C), F32)))
    o_lat = acc / l
    vt = jnp.concatenate([o_lat[:, 128 * i:128 * (i + 1)] for i in range(4)], axis=0)
    v_s[...] = vt.T

    cp_uv.wait()
    ctx = contract_c(wuv_s).astype(BF16)
    ctx_t = jnp.concatenate([ctx.astype(F32)] * 4, axis=0).T
    v_s[...] = jnp.broadcast_to(ctx_t[:, H - 1:H], (D, 128))

    s_acc = jnp.zeros((1, M), F32)
    for k in range(len(WO_MXU)):
        r0, n = wo_rows[k]
        cp_wo(k).wait()
        for h in range(r0 // D, (r0 + n) // D):
            s_acc = s_acc + jnp.dot(ctx[h:h + 1, :], wo_s[h * D:(h + 1) * D, :],
                                    preferred_element_type=F32)
    base = x + s_acc * gate

    accs = [None] * (M // 128)
    for k in range(len(WO_MXU), len(wo_rows)):
        r0, n = wo_rows[k]
        cp_wo(k).wait()
        blk = wo_s[r0:r0 + n, :].astype(F32)
        d0 = r0 - (H - 1) * D
        coef = v_s[d0:d0 + n, :]
        for j in range(M // 128):
            prod = blk[:, 128 * j:128 * (j + 1)] * coef
            parts = [prod[8 * g:8 * (g + 1), :] for g in range(n // 8)]
            if accs[j] is not None:
                parts.append(accs[j])
            while len(parts) > 1:
                nxt = [parts[a] + parts[a + 1] for a in range(0, len(parts) - 1, 2)]
                if len(parts) % 2:
                    nxt.append(parts[-1])
                parts = nxt
            accs[j] = parts[0]
    s_last = jnp.concatenate([jnp.sum(a, axis=0, keepdims=True) for a in accs], axis=1)
    o_ref[...] = (base + s_last * gate).astype(o_ref.dtype)


@jax.jit
def pallas_recurrent_scan__compressed_kv_cla__dense_activation_silu__decode_kernel(
    A_x: jax.Array,
    A_c_kv: jax.Array,
    A_w_q: jax.Array,
    A_w_uk: jax.Array,
    A_w_uv: jax.Array,
    A_w_o: jax.Array,
    B_x: jax.Array,
    B_w1: jax.Array,
    B_w2: jax.Array,
):
    del B_x
    any_spec = pl.BlockSpec(memory_space=pl.ANY)
    w_shape = (4, 128, H, D)
    out = pl.pallas_call(
        _kernel,
        in_specs=[any_spec] * 8,
        out_specs=pl.BlockSpec(memory_space=pltpu.VMEM),
        out_shape=jax.ShapeDtypeStruct((1, M), BF16),
        scratch_shapes=[
            pltpu.VMEM((1, M), BF16),
            pltpu.VMEM((SK, C), BF16),
            pltpu.VMEM(w_shape, BF16),
            pltpu.VMEM(w_shape, BF16),
            pltpu.VMEM(w_shape, BF16),
            pltpu.VMEM((H * D, M), BF16),
            pltpu.VMEM((F, M), BF16),
            pltpu.VMEM((F, M), BF16),
            pltpu.VMEM((128, 128), F32),
            pltpu.VMEM((H, C), BF16),
            pltpu.SemaphoreType.DMA((NSEM,)),
        ],
        compiler_params=pltpu.CompilerParams(
            vmem_limit_bytes=80 * 1024 * 1024,
            disable_bounds_checks=True,
            disable_semaphore_checks=True,
        ),
    )(
        A_x.reshape(1, M),
        A_c_kv.reshape(SK, C),
        A_w_q.reshape(w_shape),
        A_w_uk.reshape(w_shape),
        A_w_uv.reshape(w_shape),
        A_w_o.reshape(H * D, M),
        B_w1.T,
        B_w2,
    )
    return out.reshape(1, 1, M)
```
